```python
import jax
import jax.numpy as jnp

def _softmax(x, axis=-1):
    return jax.nn.softmax(x, axis=axis)
def _gelu(x):
    return jax.nn.gelu(x, approximate=True)
def _silu(x):
    return jax.nn.silu(x)
def _sigmoid(x):
    return jax.nn.sigmoid(x)
def _layernorm(x, axis=-1, eps=1e-5):
    m = jnp.mean(x, axis=axis, keepdims=True)
    v = jnp.var(x, axis=axis, keepdims=True)
    return (x - m) / jnp.sqrt(v + eps)
def _scatter_add(tgt, idx, src, axis=0):
    return tgt.at[idx].add(src)
def _segment_sum(src, seg, n):
    return jax.ops.segment_sum(src, seg, n)
class _Rng:
    def __init__(self, key):
        self._k = key
    def _next(self):
        self._k, sub = jax.random.split(self._k)
        return sub
    def normal(self, shape):
        return jax.random.normal(self._next(), shape, dtype=jnp.bfloat16)
    def randint(self, lo, hi, shape):
        return jax.random.randint(self._next(), shape, lo, hi, dtype=jnp.int32)
    def uniform(self, shape, lo=0.0, hi=1.0):
        return jax.random.uniform(self._next(), shape, jnp.bfloat16, lo, hi)
    def permutation(self, n):
        return jax.random.permutation(self._next(), n)


kernel_name = 'standalone__cross_network_dcn_v2__recsys'

def setup_inputs():
    _rng = _Rng(jax.random.key(int.from_bytes(__import__("os").urandom(4), "little")))
    _w = (lambda a: (lambda t: t.astype(jnp.bfloat16) if jnp.issubdtype(t.dtype, jnp.floating) else t)(jnp.asarray(a)))
    B, F, D, L = 16384, 100, 16, 3
    Din = min(F * D, 512)
    R = max(Din // 4, 2)
    sc = Din ** -0.5
    return {
        "x0": _w((lambda *s: _rng.normal(s) * 0.05)(B, Din)),
        "U":  _w((lambda *s: _rng.normal(s) * 0.05)(L, Din, R) * sc),
        "V":  _w((lambda *s: _rng.normal(s) * 0.05)(L, R, Din) * sc),
        "bs": _w((lambda *s: _rng.normal(s) * 0.05)(L, Din)),
    }

def reference(x0, U, V, bs):
    x = x0
    for l in range(U.shape[0]):
        h = jnp.einsum('rd,bd->br', V[l], x)
        h = jnp.einsum('dr,br->bd', U[l], h)
        x = x0 * (h + bs[l]) + x
    return x
```

```python
import jax
import jax.numpy as jnp
import jax.experimental.pallas as pl
import jax.experimental.pallas.tpu as pltpu

_NT = (((1,), (1,)), ((), ()))
_TM = 1024


def _kernel(x0_ref, u_ref, v_ref, b_ref, o_ref):
    xb = x0_ref[...]
    x0 = xb.astype(jnp.float32)
    x = x0
    for l in range(u_ref.shape[0]):
        h = jax.lax.dot_general(xb, v_ref[l], _NT, preferred_element_type=jnp.float32)
        y = jax.lax.dot_general(h.astype(jnp.bfloat16), u_ref[l], _NT,
                                preferred_element_type=jnp.float32)
        x = x0 * (y + b_ref[l:l + 1, :].astype(jnp.float32)) + x
        xb = x.astype(jnp.bfloat16)
    o_ref[...] = xb


@jax.jit
def pallas_standalone__cross_network_dcn_v2__recsys_kernel(
    x0: jax.Array,
    U: jax.Array,
    V: jax.Array,
    bs: jax.Array,
):
    B, D = x0.shape
    L, _, R = U.shape
    return pl.pallas_call(
        _kernel,
        grid=(B // _TM,),
        in_specs=[
            pl.BlockSpec((_TM, D), lambda i: (i, 0)),
            pl.BlockSpec((L, D, R), lambda i: (0, 0, 0)),
            pl.BlockSpec((L, R, D), lambda i: (0, 0, 0)),
            pl.BlockSpec((L, D), lambda i: (0, 0)),
        ],
        out_specs=pl.BlockSpec((_TM, D), lambda i: (i, 0)),
        out_shape=jax.ShapeDtypeStruct((B, D), x0.dtype),
        compiler_params=pltpu.CompilerParams(
            dimension_semantics=("arbitrary",),
            vmem_limit_bytes=100 * 1024 * 1024),
    )(x0, U, V, bs)
```

```python
import jax
import jax.numpy as jnp
import jax.experimental.pallas as pl
import jax.experimental.pallas.tpu as pltpu

_NT = (((1,), (1,)), ((), ()))
_F32 = jnp.float32
_BF16 = jnp.bfloat16

_PRO = (448, 960)
_SUBS = (512, 512, 512, 448, 256, 256)
_BODY = sum(_SUBS)


def _kernel(x0_hbm, u_hbm, v_hbm, b_hbm, o_hbm,
            xbuf, obuf, ubuf, vbuf, bbuf, isem, osem, wsem, rsem):
    num_rows = xbuf.shape[0]
    num_layers = ubuf.shape[0]
    n_pro = len(_PRO)
    pro_rows = sum(_PRO)
    n_loop = (num_rows - pro_rows) // _BODY
    assert pro_rows + n_loop * _BODY == num_rows

    def in_copy(off, size, k):
        return pltpu.make_async_copy(
            x0_hbm.at[pl.ds(off, size)], xbuf.at[pl.ds(off, size)], isem.at[k])

    def out_copy(off, size):
        return pltpu.make_async_copy(
            obuf.at[pl.ds(off, size)], o_hbm.at[pl.ds(off, size)], osem.at[0])

    rest = pl.ds(1, num_layers - 1)
    w_first = [
        pltpu.make_async_copy(v_hbm.at[0], vbuf.at[0], wsem.at[0]),
        pltpu.make_async_copy(u_hbm.at[0], ubuf.at[0], wsem.at[1]),
        pltpu.make_async_copy(b_hbm, bbuf, wsem.at[2]),
    ]
    w_rest = [
        pltpu.make_async_copy(v_hbm.at[rest], vbuf.at[rest], wsem.at[3]),
        pltpu.make_async_copy(u_hbm.at[rest], ubuf.at[rest], wsem.at[4]),
    ]

    def process(off, size, before_layer1=None):
        rows = pl.ds(off, size)
        xb = xbuf[rows, :]
        for l in range(num_layers):
            if l == 1 and before_layer1 is not None:
                before_layer1()
            h = jax.lax.dot_general(xb, vbuf[l], _NT, preferred_element_type=_F32)
            y = jax.lax.dot_general(h.astype(_BF16), ubuf[l], _NT,
                                    preferred_element_type=_F32)
            x0 = xbuf[rows, :].astype(_F32)
            x = x0 if l == 0 else xb.astype(_F32)
            x = x0 * (y + bbuf[l:l + 1, :].astype(_F32)) + x
            xb = x.astype(_BF16)
        obuf[rows, :] = xb

    in_copy(0, _PRO[0], 0).start()
    for c in w_first:
        c.start()
    pl.semaphore_signal(rsem, 1)
    pl.semaphore_wait(rsem, 1)
    for c in w_rest:
        c.start()

    in_copy(0, _PRO[0], 0).wait()
    for c in w_first:
        c.wait()
    off = _PRO[0]
    for i in range(1, n_pro):
        in_copy(off, _PRO[i], i).start()
        off += _PRO[i]

    def before_layer1():
        for c in w_rest:
            c.wait()
        in_copy(pro_rows, _BODY, n_pro).start()

    process(0, _PRO[0], before_layer1)
    off = _PRO[0]
    for i in range(1, n_pro):
        in_copy(off, _PRO[i], i).wait()
        process(off, _PRO[i])
        off += _PRO[i]
    out_copy(0, pro_rows).start()

    def loop(j, carry):
        base = pro_rows + j * _BODY
        in_copy(pl.multiple_of(base, 16), _BODY, n_pro + j).wait()

        @pl.when(j + 1 < n_loop)
        def _():
            in_copy(pl.multiple_of(base + _BODY, 16), _BODY, n_pro + j + 1).start()

        done = 0
        for size in _SUBS:
            start = pl.multiple_of(base + done, 16)
            process(start, size)
            out_copy(start, size).start()
            done += size
        return carry

    jax.lax.fori_loop(0, n_loop, loop, 0)
    pltpu.make_async_copy(obuf, o_hbm, osem.at[0]).wait()


@jax.jit
def pallas_standalone__cross_network_dcn_v2__recsys_kernel(
    x0: jax.Array,
    U: jax.Array,
    V: jax.Array,
    bs: jax.Array,
):
    B, D = x0.shape
    n_groups = len(_PRO) + (B - sum(_PRO)) // _BODY
    any_spec = pl.BlockSpec(memory_space=pl.ANY)
    return pl.pallas_call(
        _kernel,
        in_specs=[any_spec] * 4,
        out_specs=any_spec,
        out_shape=jax.ShapeDtypeStruct((B, D), x0.dtype),
        scratch_shapes=[
            pltpu.VMEM((B, D), x0.dtype),
            pltpu.VMEM((B, D), x0.dtype),
            pltpu.VMEM(U.shape, U.dtype),
            pltpu.VMEM(V.shape, V.dtype),
            pltpu.VMEM(bs.shape, bs.dtype),
            pltpu.SemaphoreType.DMA((n_groups,)),
            pltpu.SemaphoreType.DMA((1,)),
            pltpu.SemaphoreType.DMA((5,)),
            pltpu.SemaphoreType.REGULAR,
        ],
        compiler_params=pltpu.CompilerParams(vmem_limit_bytes=100 * 1024 * 1024),
    )(x0, U, V, bs)
```

```python
import jax
import jax.numpy as jnp
import jax.experimental.pallas as pl
import jax.experimental.pallas.tpu as pltpu

_NT = (((1,), (1,)), ((), ()))
_F32 = jnp.float32
_BF16 = jnp.bfloat16

_TILES = (256, 256, 384, 768, 1024, 640, 512, 256)
_N_RAMP = 6
_PREFETCH_AT = 3
_FIRST_OUT = 3
_EAGER_OUT = (6, 7)
_LAST_PIECES = (128, 128)

_BODY = sum(_TILES)
_STARTS = tuple(sum(_TILES[:k]) for k in range(len(_TILES)))
_RAMP_ROWS = _TILES[:_N_RAMP - 1] + (sum(_TILES[_N_RAMP - 1:]),)


def _kernel(x0_hbm, u_hbm, v_hbm, b_hbm, o_hbm,
            xbuf, obuf, ubuf, vbuf, bbuf,
            ramp_sem, next_sem, out_sem, w_sem, order_sem):
    num_rows = xbuf.shape[0]
    num_layers = ubuf.shape[0]
    n_iter = num_rows // _BODY
    assert n_iter * _BODY == num_rows

    def in_copy(off, size, sem):
        return pltpu.make_async_copy(
            x0_hbm.at[pl.ds(off, size)], xbuf.at[pl.ds(off, size)], sem)

    def ramp_copy(k):
        return in_copy(_STARTS[k], _RAMP_ROWS[k], ramp_sem.at[k])

    def out_copy(off, size):
        off = pl.multiple_of(off, 16)
        return pltpu.make_async_copy(
            obuf.at[pl.ds(off, size)], o_hbm.at[pl.ds(off, size)], out_sem.at[0])

    v_copy = [pltpu.make_async_copy(v_hbm.at[l], vbuf.at[l], w_sem.at[2 * l])
              for l in range(num_layers)]
    u_copy = [pltpu.make_async_copy(u_hbm.at[l], ubuf.at[l], w_sem.at[2 * l + 1])
              for l in range(num_layers)]
    b_copy = pltpu.make_async_copy(b_hbm, bbuf, w_sem.at[2 * num_layers])

    stages = [[ramp_copy(0), v_copy[0]], [u_copy[0], b_copy]]
    for l in range(1, num_layers):
        stages += [[v_copy[l]], [u_copy[l]]]
    stages += [[ramp_copy(k)] for k in range(1, _N_RAMP)]
    for stage in stages:
        for c in stage:
            c.start()
        pl.semaphore_signal(order_sem, 1)
        pl.semaphore_wait(order_sem, 1)

    def cross_layers(start, size, first=None, eager_out=False):
        rows = pl.ds(start, size)
        xb = xbuf[rows, :]
        for l in range(num_layers):
            if first is not None:
                pl.when(first)(v_copy[l].wait)
            h = jax.lax.dot_general(xb, vbuf[l], _NT, preferred_element_type=_F32)
            if first is not None:
                pl.when(first)(u_copy[l].wait)
                if l == 0:
                    pl.when(first)(b_copy.wait)
            y = jax.lax.dot_general(h.astype(_BF16), ubuf[l], _NT,
                                    preferred_element_type=_F32)
            x0 = xbuf[rows, :].astype(_F32)
            b = bbuf[l:l + 1, :]
            if eager_out and l == 0:
                head = pl.ds(start, 16)
                obuf[head, :] = jnp.broadcast_to(b, (16, b.shape[1]))
                b = obuf[head, :].astype(_F32)[0:1, :]
            x = x0 if l == 0 else xb.astype(_F32)
            x = x0 * (y + b.astype(_F32)) + x
            xb = x.astype(_BF16)
        return xb

    def body(j, carry):
        base = j * _BODY
        first = j == 0
        for k, size in enumerate(_TILES):
            start = pl.multiple_of(base + _STARTS[k], 16)
            if k < _N_RAMP:
                pl.when(first)(ramp_copy(k).wait)
            if k == 0:
                pl.when(j > 0)(in_copy(start, _BODY, next_sem.at[0]).wait)
            if k == _PREFETCH_AT:
                @pl.when(j + 1 < n_iter)
                def _():
                    nxt = pl.multiple_of(base + _BODY, 16)
                    in_copy(nxt, _BODY, next_sem.at[0]).start()

            xb = cross_layers(start, size, first if k == 0 else None,
                              k in _EAGER_OUT)

            if k == len(_TILES) - 1:
                done = 0
                for piece in _LAST_PIECES:
                    off = pl.multiple_of(start + done, 16)
                    obuf[pl.ds(off, piece), :] = xb[done:done + piece, :]
                    out_copy(off, piece).start()
                    done += piece
            else:
                obuf[pl.ds(start, size), :] = xb
                if k == _FIRST_OUT:
                    out_copy(base, _STARTS[k] + size).start()
                elif k > _FIRST_OUT:
                    out_copy(start, size).start()
        return carry

    jax.lax.fori_loop(0, n_iter, body, 0)
    pltpu.make_async_copy(obuf, o_hbm, out_sem.at[0]).wait()


@jax.jit
def pallas_standalone__cross_network_dcn_v2__recsys_kernel(
    x0: jax.Array,
    U: jax.Array,
    V: jax.Array,
    bs: jax.Array,
):
    B, D = x0.shape
    any_spec = pl.BlockSpec(memory_space=pl.ANY)
    return pl.pallas_call(
        _kernel,
        in_specs=[any_spec] * 4,
        out_specs=any_spec,
        out_shape=jax.ShapeDtypeStruct((B, D), x0.dtype),
        scratch_shapes=[
            pltpu.VMEM((B, D), x0.dtype),
            pltpu.VMEM((B, D), x0.dtype),
            pltpu.VMEM(U.shape, U.dtype),
            pltpu.VMEM(V.shape, V.dtype),
            pltpu.VMEM(bs.shape, bs.dtype),
            pltpu.SemaphoreType.DMA((_N_RAMP,)),
            pltpu.SemaphoreType.DMA((1,)),
            pltpu.SemaphoreType.DMA((1,)),
            pltpu.SemaphoreType.DMA((2 * U.shape[0] + 1,)),
            pltpu.SemaphoreType.REGULAR,
        ],
        compiler_params=pltpu.CompilerParams(
            vmem_limit_bytes=100 * 1024 * 1024,
            flags={"XLA_TPU_RESCHEDULE_DMA_DONES": True},
        ),
    )(x0, U, V, bs)
```
